```python
import os as _os
_os.environ.setdefault("JAX_PLATFORMS", "cpu")
import jax
import jax.numpy as jnp

def _softmax(x, axis=-1):
    return jax.nn.softmax(x, axis=axis)
def _gelu(x):
    return jax.nn.gelu(x, approximate=True)
def _silu(x):
    return jax.nn.silu(x)
def _sigmoid(x):
    return jax.nn.sigmoid(x)
def _layernorm(x, axis=-1, eps=1e-5):
    m = jnp.mean(x, axis=axis, keepdims=True)
    v = jnp.var(x, axis=axis, keepdims=True)
    return (x - m) / jnp.sqrt(v + eps)
def _scatter_add(tgt, idx, src, axis=0):
    return tgt.at[idx].add(src)
def _segment_sum(src, seg, n):
    return jax.ops.segment_sum(src, seg, n)
class _Rng:
    def __init__(self, key):
        self._k = key
    def _next(self):
        self._k, sub = jax.random.split(self._k)
        return sub
    def normal(self, shape):
        return jax.random.normal(self._next(), shape, dtype=jnp.bfloat16)
    def randint(self, lo, hi, shape):
        return jax.random.randint(self._next(), shape, lo, hi, dtype=jnp.int32)
    def uniform(self, shape, lo=0.0, hi=1.0):
        return jax.random.uniform(self._next(), shape, jnp.bfloat16, lo, hi)
    def permutation(self, n):
        return jax.random.permutation(self._next(), n)


kernel_name = 'concat_heads__sliding_local_dilated__sliding_block__prompt'

def setup_inputs():
    _rng = _Rng(jax.random.key(int.from_bytes(__import__("os").urandom(4), "little")))
    _w = (lambda a: (lambda t: t.astype(jnp.bfloat16) if jnp.issubdtype(t.dtype, jnp.floating) else t)(jnp.asarray(a)))
    def _A_setup():
        B, S, D = 1, 2048, 1024
        return {
            "x": _w((lambda *s: _rng.normal(s) * 0.2)(B, S, D)),
            "wqkv": _w((lambda *s: _rng.normal(s) * 0.2)(D, 3 * D)),
            "wo": _w((lambda *s: _rng.normal(s) * 0.05)(D, D)),
        }
    _A_in = _A_setup()

    def _B_setup():
        B, S, D = 1, 2048, 1024
        return {
            "x": _w((lambda *s: _rng.normal(s) * 0.2)(B, S, D)),
            "wqkv": _w((lambda *s: _rng.normal(s) * 0.2)(D, 3 * D)),
            "wo": _w((lambda *s: _rng.normal(s) * 0.05)(D, D)),
        }
    _B_in = _B_setup()

    return {
        "A_x": _A_in["x"],
        "A_wqkv": _A_in["wqkv"],
        "A_wo": _A_in["wo"],
        "B_x": _B_in["x"],
        "B_wqkv": _B_in["wqkv"],
        "B_wo": _B_in["wo"],
    }

def reference(A_x, A_wqkv, A_wo, B_x, B_wqkv, B_wo):
    def _A_ref(x, wqkv, wo):
        B, S, D = x.shape
        H = 32; Dh = D // H
        W, dil = 8, 2
        qkv = (lambda x, *d: x.transpose(*d))((x @ wqkv).reshape(B, S, 3, H, Dh), 2, 0, 3, 1, 4)
        q, k, v = qkv[0], qkv[1], qkv[2]
        scale = Dh ** -0.5
        pos = jnp.arange(S)
        off = jnp.arange(W) * dil
        idx = pos[:, None] - off[None, :]
        mask = idx >= 0
        idx_c = jnp.where(mask, idx, 0).reshape(-1)
        kg = k[:, :, idx_c, :].reshape(B, H, S, W, Dh)
        vg = v[:, :, idx_c, :].reshape(B, H, S, W, Dh)
        logits = jnp.einsum("bhsd,bhswd->bhsw", q, kg) * scale
        logits = jnp.where(mask[None, None, :, :], logits, -1e9)
        attn = _softmax(logits, axis=-1)
        o = jnp.einsum("bhsw,bhswd->bhsd", attn, vg)
        return (lambda x, *d: x.transpose(*d))(o, 0, 2, 1, 3).reshape(B, S, D) @ wo

    def _B_ref(x, wqkv, wo):
        B, S, D = x.shape
        H = 32; Dh = D // H; W = 256
        qkv = (lambda x, *d: x.transpose(*d))((x @ wqkv).reshape(B, S, 3, H, Dh), 2, 0, 3, 1, 4)
        q, k, v = qkv[0], qkv[1], qkv[2]
        scores = jnp.einsum("bhqd,bhkd->bhqk", q, k) * (Dh ** -0.5)
        idx = jnp.arange(S)
        mask = (idx[:, None] - idx[None, :] >= 0) & (idx[:, None] - idx[None, :] < W)
        scores = jnp.where(mask[None, None], scores, -1e9)
        p = _softmax(scores, axis=-1)
        o = jnp.einsum("bhqk,bhkd->bhqd", p, v)
        return (lambda x, *d: x.transpose(*d))(o, 0, 2, 1, 3).reshape(B, S, D) @ wo

    a = _A_ref(A_x, A_wqkv, A_wo)
    b = _B_ref(B_x, B_wqkv, B_wo)
    return jnp.concatenate([a, b], axis=-1)
```

```python
import functools
import math

import jax
import jax.numpy as jnp
import jax.experimental.pallas as pl
import jax.experimental.pallas.tpu as pltpu

H = 32
DH = 32
A_W = 8
A_DIL = 2
B_W = 256
LANES = 128
HPG = LANES // DH
NEG = -1e9

T = 256
TQ = 128
A_HALO = 16
A_PAD = 24


def _kernel(ax_ref, bx_ref, awqkv_hbm, awo_hbm, bwqkv_hbm, bwo_hbm, o_ref,
            awqkv_ref, awo_ref, bwqkv_ref, bwo_ref, sems,
            ka_scr, va_scr, kb_scr, vb_scr, *, S, D):
    i = pl.program_id(0)
    c_exp = (DH ** -0.5) * math.log2(math.e)
    G = D // LANES
    f32 = jnp.float32
    bf16 = jnp.bfloat16

    def wcopy(n):
        if n < 3:
            return pltpu.make_async_copy(awqkv_hbm.at[:, n * D:(n + 1) * D],
                                         awqkv_ref.at[:, n * D:(n + 1) * D], sems.at[n])
        if n == 3:
            return pltpu.make_async_copy(bwqkv_hbm, bwqkv_ref, sems.at[n])
        if n == 4:
            return pltpu.make_async_copy(awo_hbm, awo_ref, sems.at[n])
        return pltpu.make_async_copy(bwo_hbm, bwo_ref, sems.at[n])

    def wwait(*ns):
        @pl.when(i == 0)
        def _():
            for n in ns:
                wcopy(n).wait()

    lane = jax.lax.broadcasted_iota(jnp.int32, (1, LANES), 1)
    lane_head = lane // DH

    @pl.when(i == 0)
    def _():
        for n in range(6):
            wcopy(n).start()
        ka_scr[:, 0:A_PAD, :] = jnp.zeros((4, A_PAD, D), f32)
        va_scr[:, 0:A_PAD, :] = jnp.zeros((4, A_PAD, D), f32)
        kb_scr[0:B_W, :] = jnp.zeros((B_W, D), bf16)
        vb_scr[:, 0:B_W] = jnp.zeros((D, B_W), bf16)
        wcopy(0).wait()

    xa = ax_ref[...]
    qa = jnp.dot(xa, awqkv_ref[:, 0:D], preferred_element_type=f32)
    qa = qa.astype(bf16).astype(f32) * c_exp
    wwait(1)
    k = jnp.dot(xa, awqkv_ref[:, D:2 * D], preferred_element_type=f32)
    k = k.astype(bf16).astype(f32)
    for s in range(4):
        ka_scr[s, A_HALO + A_DIL * s:A_HALO + A_DIL * s + T, :] = k
    wwait(2)
    v = jnp.dot(xa, awqkv_ref[:, 2 * D:3 * D], preferred_element_type=f32)
    v = v.astype(bf16).astype(f32)
    for s in range(4):
        va_scr[s, A_HALO + A_DIL * s:A_HALO + A_DIL * s + T, :] = v
    wwait(3)

    xb = bx_ref[...]
    base = pl.multiple_of(B_W + i * T, T)
    qb_tiles = [None] * G

    def b_proj_tile(t):
        resf = jnp.dot(xb, bwqkv_ref[:, t * LANES:(t + 1) * LANES],
                       preferred_element_type=f32)
        res = resf.astype(bf16)
        if t < G:
            qb_tiles[t] = res
        elif t < 2 * G:
            kb_scr[pl.ds(base, T), (t - G) * LANES:(t - G + 1) * LANES] = res
        else:
            vb_scr[(t - 2 * G) * LANES:(t - 2 * G + 1) * LANES, pl.ds(base, T)] = resf.T.astype(bf16)

    r = jax.lax.broadcasted_iota(jnp.int32, (LANES, LANES), 0) // DH
    c = jax.lax.broadcasted_iota(jnp.int32, (LANES, LANES), 1) // DH
    bd = jnp.where(r == c, 1.0, 0.0).astype(bf16)

    row16 = jax.lax.broadcasted_iota(jnp.int32, (A_HALO, LANES), 0) + i * T

    def a_logits(g):
        cs = slice(g * LANES, (g + 1) * LANES)
        qg = qa[:, cs]
        lgs = []
        for w in range(A_W):
            off = A_HALO - 8 * (w // 4)
            kw = ka_scr[w % 4, off:off + T, cs]
            lgs.append(jnp.dot((qg * kw).astype(bf16), bd, preferred_element_type=f32))
        return lgs

    def a_softmax_pv(g, lgs):
        cs = slice(g * LANES, (g + 1) * LANES)
        ls = []
        for w in range(A_W):
            lw = lgs[w]
            if w > 0:
                lw = jnp.concatenate(
                    [jnp.where(row16 >= A_DIL * w, lw[0:A_HALO], NEG), lw[A_HALO:]], axis=0)
            ls.append(lw)
        m = ls[0]
        for w in range(1, A_W):
            m = jnp.maximum(m, ls[w])
        den = jnp.zeros((T, LANES), f32)
        acc = jnp.zeros((T, LANES), f32)
        for w in range(A_W):
            off = A_HALO - 8 * (w // 4)
            p = jnp.exp2(ls[w] - m)
            den = den + p
            acc = acc + p * va_scr[w % 4, off:off + T, cs]
        return (acc / den).astype(bf16)

    outs = []
    cur = a_logits(0)
    for g in range(G):
        b_proj_tile(g)
        nxt = a_logits(g + 1) if g + 1 < G else None
        b_proj_tile(G + g)
        outs.append(a_softmax_pv(g, cur))
        b_proj_tile(2 * G + g)
        cur = nxt
    oa = jnp.concatenate(outs, axis=1)
    ka_scr[:, 0:A_PAD, :] = ka_scr[:, T:T + A_PAD, :]
    va_scr[:, 0:A_PAD, :] = va_scr[:, T:T + A_PAD, :]
    wwait(4, 5)

    TK = TQ + B_W
    j = jax.lax.broadcasted_iota(jnp.int32, (TK, TQ), 0)
    a = jax.lax.broadcasted_iota(jnp.int32, (TK, TQ), 1)
    band = (j > a) & (j <= a + B_W)
    ones_rows = jnp.ones((16, TK), bf16)

    NSB = T // TQ
    units = [(sb, g) for sb in range(NSB) for g in range(G)]
    masks = [band & (j + (i * T + sb * TQ) >= B_W) for sb in range(NSB)]
    kstarts = [pl.multiple_of(i * T + sb * TQ, TQ) for sb in range(NSB)]
    outs = {}

    def scores(sb, g):
        cs = slice(g * LANES, (g + 1) * LANES)
        qg = qb_tiles[g][sb * TQ:(sb + 1) * TQ, :]
        kg = kb_scr[pl.ds(kstarts[sb], TK), cs]
        return [jax.lax.dot_general(kg, jnp.where(lane_head == h, qg, jnp.zeros_like(qg)),
                                    (((1,), (1,)), ((), ())), preferred_element_type=f32)
                for h in range(HPG)]

    def dense(u):
        sb, g = units[u]
        cs = slice(g * LANES, (g + 1) * LANES)
        if sb == 0:
            o_ref[:, cs] = jnp.dot(oa, awo_ref[:, cs],
                                   preferred_element_type=f32).astype(o_ref.dtype)
        else:
            ob = jnp.concatenate([outs[(sb - 1, gg)] for gg in range(G)], axis=1)
            o_ref[(sb - 1) * TQ:sb * TQ, D + g * LANES:D + (g + 1) * LANES] = jnp.dot(
                ob, bwo_ref[:, cs], preferred_element_type=f32).astype(o_ref.dtype)

    def softmax_pv(sb, g, sTs):
        ohs = []
        for h in range(HPG):
            sT = jnp.where(masks[sb], sTs[h], NEG)
            m = jnp.max(sT, axis=0, keepdims=True)
            pT = jnp.exp2((sT - m) * c_exp).astype(bf16)
            r0 = g * LANES + h * DH
            vT = vb_scr[r0:r0 + DH, pl.ds(kstarts[sb], TK)]
            vT = jnp.concatenate([vT, ones_rows], axis=0)
            oT = jnp.dot(vT, pT, preferred_element_type=f32)
            ohs.append(oT[0:DH] / oT[DH:DH + 1])
        og = jnp.concatenate(ohs, axis=0).T
        outs[(sb, g)] = og.astype(bf16)

    cur = scores(*units[0])
    for u in range(len(units)):
        nxt = scores(*units[u + 1]) if u + 1 < len(units) else None
        if u != G:
            dense(u)
        softmax_pv(*units[u], cur)
        if u == G - 1:
            dense(G)
        cur = nxt
    ob = jnp.concatenate([outs[(NSB - 1, gg)] for gg in range(G)], axis=1)
    o_ref[(NSB - 1) * TQ:NSB * TQ, D:2 * D] = jnp.dot(
        ob, bwo_ref[...], preferred_element_type=f32).astype(o_ref.dtype)


@jax.jit
def pallas_concat_heads__sliding_local_dilated__sliding_block__prompt_kernel(
    A_x: jax.Array,
    A_wqkv: jax.Array,
    A_wo: jax.Array,
    B_x: jax.Array,
    B_wqkv: jax.Array,
    B_wo: jax.Array,
):
    Bsz, S, D = A_x.shape
    assert Bsz == 1 and S % T == 0 and D == H * DH
    nblk = S // T
    ax = A_x.reshape(S, D)
    bx = B_x.reshape(S, D)

    anyspec = pl.BlockSpec(memory_space=pl.ANY)
    out = pl.pallas_call(
        functools.partial(_kernel, S=S, D=D),
        grid=(nblk,),
        in_specs=[
            pl.BlockSpec((T, D), lambda i: (i, 0)),
            pl.BlockSpec((T, D), lambda i: (i, 0)),
            anyspec, anyspec, anyspec, anyspec,
        ],
        out_specs=pl.BlockSpec((T, 2 * D), lambda i: (i, 0)),
        out_shape=jax.ShapeDtypeStruct((S, 2 * D), A_x.dtype),
        scratch_shapes=[
            pltpu.VMEM((D, 3 * D), jnp.bfloat16),
            pltpu.VMEM((D, D), jnp.bfloat16),
            pltpu.VMEM((D, 3 * D), jnp.bfloat16),
            pltpu.VMEM((D, D), jnp.bfloat16),
            pltpu.SemaphoreType.DMA((6,)),
            pltpu.VMEM((4, A_PAD + T, D), jnp.float32),
            pltpu.VMEM((4, A_PAD + T, D), jnp.float32),
            pltpu.VMEM((B_W + S, D), jnp.bfloat16),
            pltpu.VMEM((D, B_W + S), jnp.bfloat16),
        ],
        compiler_params=pltpu.CompilerParams(
            dimension_semantics=("arbitrary",),
            vmem_limit_bytes=100 * 1024 * 1024,
        ),
    )(ax, bx, A_wqkv, A_wo, B_wqkv, B_wo)
    return out.reshape(Bsz, S, 2 * D)
```

```python
import functools
import math

import jax
import jax.numpy as jnp
import jax.experimental.pallas as pl
import jax.experimental.pallas.tpu as pltpu

H = 32
DH = 32
A_W = 8
A_DIL = 2
B_W = 256
LANES = 128
HPG = LANES // DH
NEG = -1e9

T = 256
TQ = 128
A_HALO = 16
A_PAD = 24


def _kernel(ax_ref, bx_ref, awqkv_hbm, awo_hbm, bwqkv_hbm, bwo_hbm, o_ref,
            awqkv_ref, awo_ref, bwqkv_ref, bwo_ref, sems,
            ka_scr, va_scr, kb_scr, vb_scr, *, S, D):
    i = pl.program_id(0)
    c_exp = (DH ** -0.5) * math.log2(math.e)
    G = D // LANES
    f32 = jnp.float32
    bf16 = jnp.bfloat16

    def wcopy(n):
        if n < 3:
            return pltpu.make_async_copy(awqkv_hbm.at[:, n * D:(n + 1) * D],
                                         awqkv_ref.at[:, n * D:(n + 1) * D], sems.at[n])
        if n < 6:
            m = n - 3
            return pltpu.make_async_copy(bwqkv_hbm.at[:, m * D:(m + 1) * D],
                                         bwqkv_ref.at[:, m * D:(m + 1) * D], sems.at[n])
        if n == 6:
            return pltpu.make_async_copy(awo_hbm, awo_ref, sems.at[n])
        return pltpu.make_async_copy(bwo_hbm, bwo_ref, sems.at[n])

    def wwait(*ns):
        @pl.when(i == 0)
        def _():
            for n in ns:
                wcopy(n).wait()

    lane = jax.lax.broadcasted_iota(jnp.int32, (1, LANES), 1)
    lane_head = lane // DH

    @pl.when(i == 0)
    def _():
        for n in range(8):
            wcopy(n).start()
        ka_scr[:, 0:A_PAD, :] = jnp.zeros((4, A_PAD, D), f32)
        va_scr[:, 0:A_PAD, :] = jnp.zeros((4, A_PAD, D), f32)
        ka_scr[:, T:T + A_PAD, :] = jnp.zeros((4, A_PAD, D), f32)
        va_scr[:, T:T + A_PAD, :] = jnp.zeros((4, A_PAD, D), f32)
        kb_scr[0:B_W, :] = jnp.zeros((B_W, D), bf16)
        vb_scr[:, 0:B_W] = jnp.zeros((D, B_W), bf16)
        wcopy(0).wait()

    xa = ax_ref[...]
    qa = jnp.dot(xa, awqkv_ref[:, 0:D], preferred_element_type=f32)
    qa = qa.astype(bf16).astype(f32) * c_exp
    wwait(1)
    k = jnp.dot(xa, awqkv_ref[:, D:2 * D], preferred_element_type=f32)
    k = k.astype(bf16).astype(f32)
    for s in range(4):
        ka_scr[s, A_HALO + A_DIL * s:A_HALO + A_DIL * s + T, :] = k
    wwait(2)
    v = jnp.dot(xa, awqkv_ref[:, 2 * D:3 * D], preferred_element_type=f32)
    v = v.astype(bf16).astype(f32)
    for s in range(4):
        va_scr[s, A_HALO + A_DIL * s:A_HALO + A_DIL * s + T, :] = v
    wwait(3)

    xb = bx_ref[...]
    base = pl.multiple_of(B_W + i * T, T)
    qb_tiles = [None] * G

    def b_proj_tile(t):
        resf = jnp.dot(xb, bwqkv_ref[:, t * LANES:(t + 1) * LANES],
                       preferred_element_type=f32)
        res = resf.astype(bf16)
        if t < G:
            qb_tiles[t] = (resf * c_exp).astype(bf16)
        elif t < 2 * G:
            kb_scr[pl.ds(base, T), (t - G) * LANES:(t - G + 1) * LANES] = res
        else:
            vb_scr[(t - 2 * G) * LANES:(t - 2 * G + 1) * LANES, pl.ds(base, T)] = resf.T.astype(bf16)

    er = jax.lax.broadcasted_iota(jnp.int32, (16, LANES), 0)
    ec = jax.lax.broadcasted_iota(jnp.int32, (16, LANES), 1) // DH
    esel = jnp.where(er == ec, 1.0, 0.0).astype(bf16)
    tok = jax.lax.broadcasted_iota(jnp.int32, (8, T), 1) + i * T

    def a_logits(g):
        cs = slice(g * LANES, (g + 1) * LANES)
        qg = qa[:, cs]
        lgs = []
        for w in range(A_W):
            off = A_HALO - 8 * (w // 4)
            kw = ka_scr[w % 4, off:off + T, cs]
            lT = jax.lax.dot_general(esel, (qg * kw).astype(bf16), (((1,), (1,)), ((), ())),
                                     preferred_element_type=f32)
            lgs.append(lT[0:8])
        return lgs

    def a_softmax_pv(g, lgs):
        cs = slice(g * LANES, (g + 1) * LANES)
        ls = []
        for w in range(A_W):
            lw = lgs[w]
            if w > 0:
                lw = jnp.where(tok >= A_DIL * w, lw, NEG)
            ls.append(lw)
        m = ls[0]
        for w in range(1, A_W):
            m = jnp.maximum(m, ls[w])
        ps = [jnp.exp2(ls[w] - m) for w in range(A_W)]
        den = ps[0]
        for w in range(1, A_W):
            den = den + ps[w]
        inv = 1.0 / den
        acc = jnp.zeros((T, LANES), f32)
        for w in range(A_W):
            off = A_HALO - 8 * (w // 4)
            pn = (ps[w] * inv)[0:HPG]
            pe = jnp.broadcast_to(pn[:, None, :], (HPG, DH, T)).reshape(LANES, T).T
            acc = acc + pe * va_scr[w % 4, off:off + T, cs]
        return acc.astype(bf16)

    outs = []
    cur = a_logits(0)
    for g in range(G):
        if g == 2:
            wwait(4)
        if g == 5:
            wwait(5)
        b_proj_tile(3 * g)
        nxt = a_logits(g + 1) if g + 1 < G else None
        b_proj_tile(3 * g + 1)
        outs.append(a_softmax_pv(g, cur))
        b_proj_tile(3 * g + 2)
        cur = nxt
    oa = jnp.concatenate(outs, axis=1)
    ka_scr[:, 0:A_PAD, :] = ka_scr[:, T:T + A_PAD, :]
    va_scr[:, 0:A_PAD, :] = va_scr[:, T:T + A_PAD, :]
    wwait(6, 7)

    TK = TQ + B_W
    j = jax.lax.broadcasted_iota(jnp.int32, (TK, TQ), 0)
    a = jax.lax.broadcasted_iota(jnp.int32, (TK, TQ), 1)
    band = (j > a) & (j <= a + B_W)
    ones_rows = jnp.ones((16, TK), bf16)

    NSB = T // TQ
    units = [(sb, g) for sb in range(NSB) for g in range(G)]
    masks = [band & (j + (i * T + sb * TQ) >= B_W) for sb in range(NSB)]
    kstarts = [pl.multiple_of(i * T + sb * TQ, TQ) for sb in range(NSB)]
    outs = {}

    def scores(sb, g):
        cs = slice(g * LANES, (g + 1) * LANES)
        qg = qb_tiles[g][sb * TQ:(sb + 1) * TQ, :]
        kg = kb_scr[pl.ds(kstarts[sb], TK), cs]
        return [jax.lax.dot_general(kg, jnp.where(lane_head == h, qg, jnp.zeros_like(qg)),
                                    (((1,), (1,)), ((), ())), preferred_element_type=f32)
                for h in range(HPG)]

    def dense(u):
        sb, g = units[u]
        cs = slice(g * LANES, (g + 1) * LANES)
        if sb == 0:
            o_ref[:, cs] = jnp.dot(oa, awo_ref[:, cs],
                                   preferred_element_type=f32).astype(o_ref.dtype)
        else:
            ob = jnp.concatenate([outs[(sb - 1, gg)] for gg in range(G)], axis=1)
            o_ref[(sb - 1) * TQ:sb * TQ, D + g * LANES:D + (g + 1) * LANES] = jnp.dot(
                ob, bwo_ref[:, cs], preferred_element_type=f32).astype(o_ref.dtype)

    def softmax_pv(sb, g, sTs):
        ohs = []
        for h in range(HPG):
            sT = jnp.where(masks[sb], sTs[h], NEG)
            m = jnp.max(sT, axis=0, keepdims=True)
            pT = jnp.exp2(sT - m).astype(bf16)
            r0 = g * LANES + h * DH
            vT = vb_scr[r0:r0 + DH, pl.ds(kstarts[sb], TK)]
            vT = jnp.concatenate([vT, ones_rows], axis=0)
            oT = jnp.dot(vT, pT, preferred_element_type=f32)
            ohs.append(oT[0:DH] / oT[DH:DH + 1])
        og = jnp.concatenate(ohs, axis=0).T
        outs[(sb, g)] = og.astype(bf16)

    cur = scores(*units[0])
    for u in range(len(units)):
        nxt = scores(*units[u + 1]) if u + 1 < len(units) else None
        if u != G:
            dense(u)
        softmax_pv(*units[u], cur)
        if u == G - 1:
            dense(G)
        cur = nxt
    ob = jnp.concatenate([outs[(NSB - 1, gg)] for gg in range(G)], axis=1)
    o_ref[(NSB - 1) * TQ:NSB * TQ, D:2 * D] = jnp.dot(
        ob, bwo_ref[...], preferred_element_type=f32).astype(o_ref.dtype)


@jax.jit
def pallas_concat_heads__sliding_local_dilated__sliding_block__prompt_kernel(
    A_x: jax.Array,
    A_wqkv: jax.Array,
    A_wo: jax.Array,
    B_x: jax.Array,
    B_wqkv: jax.Array,
    B_wo: jax.Array,
):
    Bsz, S, D = A_x.shape
    assert Bsz == 1 and S % T == 0 and D == H * DH
    nblk = S // T
    ax = A_x.reshape(S, D)
    bx = B_x.reshape(S, D)

    anyspec = pl.BlockSpec(memory_space=pl.ANY)
    out = pl.pallas_call(
        functools.partial(_kernel, S=S, D=D),
        grid=(nblk,),
        in_specs=[
            pl.BlockSpec((T, D), lambda i: (i, 0)),
            pl.BlockSpec((T, D), lambda i: (i, 0)),
            anyspec, anyspec, anyspec, anyspec,
        ],
        out_specs=pl.BlockSpec((T, 2 * D), lambda i: (i, 0)),
        out_shape=jax.ShapeDtypeStruct((S, 2 * D), A_x.dtype),
        scratch_shapes=[
            pltpu.VMEM((D, 3 * D), jnp.bfloat16),
            pltpu.VMEM((D, D), jnp.bfloat16),
            pltpu.VMEM((D, 3 * D), jnp.bfloat16),
            pltpu.VMEM((D, D), jnp.bfloat16),
            pltpu.SemaphoreType.DMA((8,)),
            pltpu.VMEM((4, A_PAD + T, D), jnp.float32),
            pltpu.VMEM((4, A_PAD + T, D), jnp.float32),
            pltpu.VMEM((B_W + S, D), jnp.bfloat16),
            pltpu.VMEM((D, B_W + S), jnp.bfloat16),
        ],
        compiler_params=pltpu.CompilerParams(
            dimension_semantics=("arbitrary",),
            vmem_limit_bytes=100 * 1024 * 1024,
        ),
    )(ax, bx, A_wqkv, A_wo, B_wqkv, B_wo)
    return out.reshape(Bsz, S, 2 * D)
```
